```python
import jax
import jax.numpy as jnp

def _softmax(x, axis=-1):
    return jax.nn.softmax(x, axis=axis)

def _gelu(x):
    return jax.nn.gelu(x, approximate=True)

def _silu(x):
    return jax.nn.silu(x)

def _sigmoid(x):
    return jax.nn.sigmoid(x)

def _layernorm(x, axis=-1, eps=1e-05):
    m = jnp.mean(x, axis=axis, keepdims=True)
    v = jnp.var(x, axis=axis, keepdims=True)
    return (x - m) / jnp.sqrt(v + eps)

def _scatter_add(tgt, idx, src, axis=0):
    return tgt.at[idx].add(src)

def _segment_sum(src, seg, n):
    return jax.ops.segment_sum(src, seg, n)

class _Rng:

    def __init__(self, key):
        self._k = key

    def _next(self):
        self._k, sub = jax.random.split(self._k)
        return sub

    def normal(self, shape):
        return jax.random.normal(self._next(), shape, dtype=jnp.bfloat16)

    def randint(self, lo, hi, shape):
        return jax.random.randint(self._next(), shape, lo, hi, dtype=jnp.int32)

    def uniform(self, shape, lo=0.0, hi=1.0):
        return jax.random.uniform(self._next(), shape, jnp.bfloat16, lo, hi)

    def permutation(self, n):
        return jax.random.permutation(self._next(), n)
kernel_name = 'adaLN_cond__compressed_kv_cla__dense_activation_relu__decode'

def setup_inputs():
    _rng = _Rng(jax.random.key(int.from_bytes(__import__("os").urandom(4), "little")))
    _w = lambda a: (lambda t: t.astype(jnp.bfloat16) if jnp.issubdtype(t.dtype, jnp.floating) else t)(jnp.asarray(a))

    def _A_setup():
        B, H, Sq, Sk, D, M = (8, 32, 1, 4096, 128, 512)
        Dc = 4 * D
        return {'x': _w((lambda *s: _rng.normal(s) * 0.05)(B, Sq, M)), 'c_kv': _w((lambda *s: _rng.normal(s) * 0.05)(B, Sk, Dc)), 'w_q': _w((lambda *s: _rng.normal(s) * 0.05)(M, H, D) * M ** (-0.5)), 'w_uk': _w((lambda *s: _rng.normal(s) * 0.05)(Dc, H, D) * Dc ** (-0.5)), 'w_uv': _w((lambda *s: _rng.normal(s) * 0.05)(Dc, H, D) * Dc ** (-0.5)), 'w_o': _w((lambda *s: _rng.normal(s) * 0.05)(H, D, M) * (H * D) ** (-0.5))}
    _A_in = _A_setup()

    def _B_setup():
        B, S, D, Dff = (8, 1, 512, 1792)
        return {'x': _w((lambda *s: _rng.normal(s) * 0.05)(B, S, D)), 'w1': _w((lambda *s: _rng.normal(s) * 0.05)(D, Dff)), 'w2': _w((lambda *s: _rng.normal(s) * 0.05)(Dff, D))}
    _B_in = _B_setup()
    return {'A_x': _A_in['x'], 'A_c_kv': _A_in['c_kv'], 'A_w_q': _A_in['w_q'], 'A_w_uk': _A_in['w_uk'], 'A_w_uv': _A_in['w_uv'], 'A_w_o': _A_in['w_o'], 'B_x': _B_in['x'], 'B_w1': _B_in['w1'], 'B_w2': _B_in['w2'], 'c': _w((lambda *s: _rng.normal(s) * 0.05)(8, 512)), 'w_mod': _w((lambda *s: _rng.normal(s) * 0.05)(512, 6 * 512) * 512 ** (-0.5))}

def reference(A_x, A_c_kv, A_w_q, A_w_uk, A_w_uv, A_w_o, B_x, B_w1, B_w2, c, w_mod):

    def _A_ref(x, c_kv, w_q, w_uk, w_uv, w_o):
        B, Sq, M = (x.shape[0], x.shape[1], x.shape[2])
        Sk = c_kv.shape[1]
        H, D = (w_q.shape[1], w_q.shape[2])
        q = jnp.einsum('bqm,mhd->bhqd', x, w_q)
        k = jnp.einsum('bkc,chd->bhkd', c_kv, w_uk)
        v = jnp.einsum('bkc,chd->bhkd', c_kv, w_uv)
        scores = jnp.einsum('bhqd,bhkd->bhqk', q, k) * D ** (-0.5)
        off = Sk - Sq
        qi = jnp.arange(Sq)[:, None]
        kj = jnp.arange(Sk)[None, :]
        cmask = kj <= qi + off
        scores = jnp.where(cmask[None, None], scores, -1000000000.0)
        p = _softmax(scores, axis=-1)
        ctx = jnp.einsum('bhqk,bhkd->bhqd', p, v)
        return jnp.einsum('bhqd,hdm->bqm', ctx, w_o)

    def _B_ref(x, w1, w2):
        h = jnp.einsum('bsd,df->bsf', x, w1)
        zero = jnp.zeros_like(h)
        h = jnp.maximum(h, zero)
        return jnp.einsum('bsf,fd->bsd', h, w2)
    x = A_x
    mod = (_silu(c) @ w_mod).reshape(c.shape[0], 6, 1, -1)
    sa, ca, ga, sb, cb, gb = (mod[:, 0].copy(), mod[:, 1].copy(), mod[:, 2].copy(), mod[:, 3].copy(), mod[:, 4].copy(), mod[:, 5].copy())
    h = _layernorm(x, axis=-1) * (1 + ca) + sa
    x = x + ga * _A_ref(h, A_c_kv, A_w_q, A_w_uk, A_w_uv, A_w_o)
    h = _layernorm(x, axis=-1) * (1 + cb) + sb
    x = x + gb * _B_ref(h, B_w1, B_w2)
    return x
```

```python
import jax
import jax.numpy as jnp
from jax import lax
import jax.experimental.pallas as pl
import jax.experimental.pallas.tpu as pltpu

CFG = dict(win=100, kvc=1, compute=True)
B, H, SK, D, M, DC, DFF = 8, 32, 4096, 128, 512, 512, 1792
F32, BF16, U32 = jnp.float32, jnp.bfloat16, jnp.uint32
NT = (((1,), (1,)), ((), ()))


def _dot(a, b):
    return jnp.dot(a, b, preferred_element_type=F32)


def _dot_nt(a, b):
    return lax.dot_general(a, b, NT, preferred_element_type=F32)


def _ln(x):
    m = jnp.mean(x, axis=-1, keepdims=True)
    d = x - m
    v = jnp.mean(d * d, axis=-1, keepdims=True)
    return d * lax.rsqrt(v + 1e-5)


def _pair(w_ref, blk, j):
    w32 = w_ref.bitcast(U32)
    w = w32[pl.ds(blk * 128 * 16 + j, 128, stride=16), :]
    lo = lax.bitcast_convert_type(w << 16, F32).astype(BF16)
    hi = lax.bitcast_convert_type(w & U32(0xFFFF0000), F32).astype(BF16)
    return lo, hi


def _kernel(x_hbm, c_hbm, kv_hbm, wq_hbm, wuk_hbm, wuv_hbm, wo_hbm, w1_hbm, w2_hbm, wm_hbm, o_ref,
            x_v, c_v, kv_v, wq_v, wuk_v, wuv_v, wo_v, w1_v, w2_v, wm_v, qa_s, cc_s, sems):
    copies = []

    def add(src, dst):
        copies.append(pltpu.make_async_copy(src, dst, sems.at[len(copies)]))
        return len(copies) - 1

    id_wm0 = add(wm_hbm.at[:, 0:1024], wm_v.at[:, 0:1024])
    id_c = add(c_hbm, c_v)
    id_x = add(x_hbm, x_v)
    id_wq = [add(wq_hbm.at[pl.ds(i * 4096, 4096)], wq_v.at[pl.ds(i * 4096, 4096)]) for i in range(4)]
    id_wuk = [add(wuk_hbm.at[pl.ds(i * 4096, 4096)], wuk_v.at[pl.ds(i * 4096, 4096)]) for i in range(4)]
    kc = CFG['kvc']
    kr = SK // kc
    id_kv = [[add(kv_hbm.at[b, pl.ds(i * kr, kr)], kv_v.at[b, pl.ds(i * kr, kr)]) for i in range(kc)] for b in range(B)]
    id_wuv = [add(wuv_hbm.at[pl.ds(i * 4096, 4096)], wuv_v.at[pl.ds(i * 4096, 4096)]) for i in range(4)]
    id_wo = [add(wo_hbm.at[pl.ds(i * 1024, 1024)], wo_v.at[pl.ds(i * 1024, 1024)]) for i in range(4)]
    id_wm1 = add(wm_hbm.at[:, 1024:3072], wm_v.at[:, 1024:3072])
    id_w1 = add(w1_hbm, w1_v)
    id_w2 = [add(w2_hbm.at[pl.ds(i * 256, 256)], w2_v.at[pl.ds(i * 256, 256)]) for i in range(7)]
    st = dict(started=0, waited=0)

    def start_upto(n):
        while st['started'] < min(n, len(copies)):
            copies[st['started']].start()
            st['started'] += 1

    def wait(i):
        while st['waited'] <= i:
            start_upto(st['waited'] + CFG['win'])
            copies[st['waited']].wait()
            st['waited'] += 1
        start_upto(st['waited'] + CFG['win'])

    if not CFG['compute']:
        wait(len(copies) - 1)
        o_ref[...] = x_v[...]
        return

    wait(id_x)
    cf = c_v[...].astype(F32)
    sc = (cf * jax.nn.sigmoid(cf)).astype(BF16)
    mod0 = _dot(sc, wm_v[:, 0:1024])
    x = x_v[...].astype(F32)
    h = (_ln(x) * (1.0 + mod0[:, 512:1024]) + mod0[:, 0:512]).astype(BF16)

    q = [None] * H
    for blk in range(4):
        wait(id_wq[blk])
        hb = h[:, blk * 128:(blk + 1) * 128]
        for j in range(H // 2):
            for p, w in enumerate(_pair(wq_v, blk, j)):
                t = _dot(hb, w)
                q[2 * j + p] = t if blk == 0 else q[2 * j + p] + t
    q = [(t * (D ** -0.5)).astype(BF16) for t in q]
    for blk in range(4):
        wait(id_wuk[blk])
        for j in range(H // 2):
            for p, w in enumerate(_pair(wuk_v, blk, j)):
                hh = 2 * j + p
                qa_s[blk, pl.ds(hh * 8, 8), :] = _dot_nt(q[hh], w)

    for b in range(B):
        wait(id_kv[b][-1])
        qa = jnp.concatenate([qa_s[blk, pl.ds(b, H, stride=8), :] for blk in range(4)], axis=1).astype(BF16)
        s = _dot_nt(qa, kv_v[b])
        m = jnp.max(s, axis=-1, keepdims=True)
        p = jnp.exp(s - m)
        l = jnp.sum(p, axis=-1, keepdims=True)
        cc = _dot(p.astype(BF16), kv_v[b]) * (1.0 / l)
        for blk in range(4):
            cc_s[blk, pl.ds(b * H, H), :] = cc[:, blk * 128:(blk + 1) * 128]

    ctx = [None] * H
    for blk in range(4):
        wait(id_wuv[blk])
        for j in range(H // 2):
            for p, w in enumerate(_pair(wuv_v, blk, j)):
                hh = 2 * j + p
                t = _dot(cc_s[blk, pl.ds(hh, B, stride=H), :].astype(BF16), w)
                ctx[hh] = t if blk == 0 else ctx[hh] + t
    att = None
    for blk in range(4):
        wait(id_wo[blk])
        cb = jnp.concatenate(ctx[blk * 8:(blk + 1) * 8], axis=1).astype(BF16)
        t = _dot(cb, wo_v[pl.ds(blk * 1024, 1024), :])
        att = t if att is None else att + t
    wait(id_wm1)
    mod1 = _dot(sc, wm_v[:, 1024:3072])
    x1 = x + mod1[:, 0:512] * att
    h2 = (_ln(x1) * (1.0 + mod1[:, 1024:1536]) + mod1[:, 512:1024]).astype(BF16)
    wait(id_w1)
    a = jnp.maximum(_dot(h2, w1_v[...]), 0.0).astype(BF16)
    y = None
    for i in range(7):
        wait(id_w2[i])
        t = _dot(a[:, i * 256:(i + 1) * 256], w2_v[pl.ds(i * 256, 256), :])
        y = t if y is None else y + t
    o_ref[...] = (x1 + mod1[:, 1536:2048] * y).astype(o_ref.dtype)


@jax.jit
def pallas_adaLN_cond__compressed_kv_cla__dense_activation_relu__decode_kernel(
        A_x, A_c_kv, A_w_q, A_w_uk, A_w_uv, A_w_o, B_x, B_w1, B_w2, c, w_mod):
    del B_x
    hbm = pl.BlockSpec(memory_space=pl.ANY)
    out = pl.pallas_call(
        _kernel,
        in_specs=[hbm] * 10,
        out_specs=pl.BlockSpec(memory_space=pltpu.VMEM),
        out_shape=jax.ShapeDtypeStruct((B, M), A_x.dtype),
        scratch_shapes=[
            pltpu.VMEM((B, M), BF16), pltpu.VMEM((B, M), BF16), pltpu.VMEM((B, SK, DC), BF16),
            pltpu.VMEM((M * H, D), BF16), pltpu.VMEM((DC * H, D), BF16), pltpu.VMEM((DC * H, D), BF16),
            pltpu.VMEM((H * D, M), BF16), pltpu.VMEM((M, DFF), BF16), pltpu.VMEM((DFF, M), BF16),
            pltpu.VMEM((M, 6 * M), BF16),
            pltpu.VMEM((4, B * H, 128), F32), pltpu.VMEM((4, B * H, 128), F32),
            pltpu.SemaphoreType.DMA((128,)),
        ],
        compiler_params=pltpu.CompilerParams(vmem_limit_bytes=100 * 1024 * 1024),
    )(A_x.reshape(B, M), c, A_c_kv, A_w_q.reshape(M * H, D), A_w_uk.reshape(DC * H, D),
      A_w_uv.reshape(DC * H, D), A_w_o.reshape(H * D, M), B_w1, B_w2, w_mod)
    return out.reshape(B, 1, M)
```

```python
import jax
import jax.numpy as jnp
from jax import lax
import jax.experimental.pallas as pl
import jax.experimental.pallas.tpu as pltpu

CFG = dict(rows=32, ns=4, unit=32, ahead=64, alt=True, compute=True, w2=(0, 1024, 1536, 1792))
NSEM = 5
B, H, SK, D, M, DC, DFF = 8, 32, 4096, 128, 512, 512, 1792
F32, BF16, U32 = jnp.float32, jnp.bfloat16, jnp.uint32
NT = (((1,), (1,)), ((), ()))


def _dot(a, b):
    return jnp.dot(a, b, preferred_element_type=F32)


def _dot_nt(a, b):
    return lax.dot_general(a, b, NT, preferred_element_type=F32)


def _ln(x):
    m = jnp.mean(x, axis=-1, keepdims=True)
    d = x - m
    v = jnp.mean(d * d, axis=-1, keepdims=True)
    return d * lax.rsqrt(v + 1e-5)


def _pair(w_ref, blk, j):
    w32 = w_ref.bitcast(U32)
    w = w32[pl.ds(blk * 128 * 16 + j, 128, stride=16), :]
    lo = lax.bitcast_convert_type(w << 16, F32).astype(BF16)
    hi = lax.bitcast_convert_type(w & U32(0xFFFF0000), F32).astype(BF16)
    return lo, hi


def _kernel(x_hbm, c_hbm, kv_hbm, wq_hbm, wuk_hbm, wuv_hbm, wo_hbm, w1_hbm, w2_hbm, wm_hbm, o_ref,
            x_v, c_v, kv_v, wq_v, wuk_v, wuv_v, wo_v, w1_v, w2_v, wm0_v, wm1_v, qa_s, cc_s, sems):
    groups = []
    pieces = []

    def add(src, dst, rows, col_parts=1, ns=CFG['ns']):
        sem = sems.at[len(groups) % NSEM]
        n_r, n_c = src.shape
        w = n_c // col_parts
        ps = [(r * rows, c * w) for r in range(n_r // rows) for c in range(col_parts)]
        n = len(ps)
        ns = ns if n % ns == 0 else 1
        lo = len(pieces)
        for k in range(n):
            r, c = ps[(k % ns) * (n // ns) + k // ns]
            pieces.append(pltpu.make_async_copy(src.at[pl.ds(r, rows), pl.ds(c, w)], dst.at[pl.ds(r, rows), pl.ds(c, w)], sem))
        groups.append((lo, len(pieces), pltpu.make_async_copy(dst, dst, sem)))
        return len(groups) - 1

    R = CFG['rows']
    id_c = add(c_hbm, c_v, B)
    id_x = add(x_hbm, x_v, B)
    id_wm0 = add(wm_hbm.at[:, 0:1024], wm0_v, R // 2)
    id_wq = add(wq_hbm, wq_v, 4 * R)
    id_wuk = add(wuk_hbm, wuk_v, 4 * R)
    id_kv = [add(kv_hbm.at[b], kv_v.at[b], R) for b in range(B)]
    id_wuv = add(wuv_hbm, wuv_v, 4 * R)
    id_wo = add(wo_hbm, wo_v, R)
    id_wm1 = add(wm_hbm.at[:, 1024:3072], wm1_v, R // 2, 2)
    id_w1 = add(w1_hbm, w1_v, R // 2, 2)
    w2_cuts = CFG['w2']
    id_w2 = [add(w2_hbm.at[lo:hi], w2_v.at[lo:hi], R, ns=2) for lo, hi in zip(w2_cuts[:-1], w2_cuts[1:])]
    st = dict(started=0, waited=0)

    def issue_upto(n):
        g_lim = st['waited'] + NSEM
        if g_lim < len(groups):
            n = min(n, groups[g_lim][0])
        while st['started'] < min(n, len(pieces)):
            pieces[st['started']].start(priority=st['started'] % 2 if CFG['alt'] else 0)
            st['started'] += 1

    def issue(n=CFG['unit']):
        issue_upto(st['started'] + n)

    def wait(g):
        while st['waited'] <= g:
            issue_upto(groups[st['waited']][1] + CFG['ahead'])
            groups[st['waited']][2].wait()
            st['waited'] += 1

    if not CFG['compute']:
        wait(len(groups) - 1)
        o_ref[...] = x_v[...]
        return

    wait(id_x)
    cf = c_v[...].astype(F32)
    sc = (cf * jax.nn.sigmoid(cf)).astype(BF16)
    x = x_v[...].astype(F32)
    xn = _ln(x)
    wait(id_wm0)
    mod0 = _dot(sc, wm0_v[...])
    h = (xn * (1.0 + mod0[:, 512:1024]) + mod0[:, 0:512]).astype(BF16)

    wait(id_wq)
    q = [None] * H
    for blk in range(4):
        hb = h[:, blk * 128:(blk + 1) * 128]
        for j in range(H // 2):
            for p, w in enumerate(_pair(wq_v, blk, j)):
                t = _dot(hb, w)
                q[2 * j + p] = t if blk == 0 else q[2 * j + p] + t
        issue()
    q = [(t * (D ** -0.5)).astype(BF16) for t in q]
    wait(id_wuk)
    for blk in range(4):
        for j in range(H // 2):
            for p, w in enumerate(_pair(wuk_v, blk, j)):
                hh = 2 * j + p
                qa_s[blk, pl.ds(hh * 8, 8), :] = _dot_nt(q[hh], w)
        issue()

    HS = SK // 2
    for b in range(B):
        wait(id_kv[b])
        qa = jnp.concatenate([qa_s[blk, pl.ds(b, H, stride=8), :] for blk in range(4)], axis=1).astype(BF16)
        s0 = _dot_nt(qa, kv_v[b, 0:HS])
        issue()
        s1 = _dot_nt(qa, kv_v[b, HS:SK])
        issue()
        m = jnp.maximum(jnp.max(s0, axis=-1, keepdims=True), jnp.max(s1, axis=-1, keepdims=True))
        p0 = jnp.exp(s0 - m)
        cc = _dot(p0.astype(BF16), kv_v[b, 0:HS])
        issue()
        p1 = jnp.exp(s1 - m)
        cc = cc + _dot(p1.astype(BF16), kv_v[b, HS:SK])
        l = jnp.sum(p0, axis=-1, keepdims=True) + jnp.sum(p1, axis=-1, keepdims=True)
        cc = cc * (1.0 / l)
        for blk in range(4):
            cc_s[blk, pl.ds(b * H, H), :] = cc[:, blk * 128:(blk + 1) * 128]
        issue()

    wait(id_wuv)
    ctx = [None] * H
    for blk in range(4):
        for j in range(H // 2):
            for p, w in enumerate(_pair(wuv_v, blk, j)):
                hh = 2 * j + p
                t = _dot(cc_s[blk, pl.ds(hh, B, stride=H), :].astype(BF16), w)
                ctx[hh] = t if blk == 0 else ctx[hh] + t
        issue()
    wait(id_wo)
    att = None
    for blk in range(2):
        cb = jnp.concatenate(ctx[blk * 16:(blk + 1) * 16], axis=1).astype(BF16)
        t = _dot(cb, wo_v[pl.ds(blk * 2048, 2048), :])
        att = t if att is None else att + t
        issue()
    wait(id_wm1)
    mod1 = _dot(sc, wm1_v[...])
    x1 = x + mod1[:, 0:512] * att
    h2 = (_ln(x1) * (1.0 + mod1[:, 1024:1536]) + mod1[:, 512:1024]).astype(BF16)
    wait(id_w1)
    a = jnp.maximum(_dot(h2, w1_v[...]), 0.0).astype(BF16)
    y = None
    for i, (lo, hi) in enumerate(zip(w2_cuts[:-1], w2_cuts[1:])):
        wait(id_w2[i])
        t = _dot(a[:, lo:hi], w2_v[lo:hi, :])
        y = t if y is None else y + t
    o_ref[...] = (x1 + mod1[:, 1536:2048] * y).astype(o_ref.dtype)


@jax.jit
def pallas_adaLN_cond__compressed_kv_cla__dense_activation_relu__decode_kernel(
        A_x, A_c_kv, A_w_q, A_w_uk, A_w_uv, A_w_o, B_x, B_w1, B_w2, c, w_mod):
    del B_x
    hbm = pl.BlockSpec(memory_space=pl.ANY)
    out = pl.pallas_call(
        _kernel,
        in_specs=[hbm] * 10,
        out_specs=pl.BlockSpec(memory_space=pltpu.VMEM),
        out_shape=jax.ShapeDtypeStruct((B, M), A_x.dtype),
        scratch_shapes=[
            pltpu.VMEM((B, M), BF16), pltpu.VMEM((B, M), BF16), pltpu.VMEM((B, SK, DC), BF16),
            pltpu.VMEM((M * H, D), BF16), pltpu.VMEM((DC * H, D), BF16), pltpu.VMEM((DC * H, D), BF16),
            pltpu.VMEM((H * D, M), BF16), pltpu.VMEM((M, DFF), BF16), pltpu.VMEM((DFF, M), BF16),
            pltpu.VMEM((M, 2 * M), BF16), pltpu.VMEM((M, 4 * M), BF16),
            pltpu.VMEM((4, B * H, 128), F32), pltpu.VMEM((4, B * H, 128), F32),
            pltpu.SemaphoreType.DMA((NSEM,)),
        ],
        compiler_params=pltpu.CompilerParams(vmem_limit_bytes=100 * 1024 * 1024),
    )(A_x.reshape(B, M), c, A_c_kv, A_w_q.reshape(M * H, D), A_w_uk.reshape(DC * H, D),
      A_w_uv.reshape(DC * H, D), A_w_o.reshape(H * D, M), B_w1, B_w2, w_mod)
    return out.reshape(B, 1, M)
```

```python
import jax
import jax.numpy as jnp
from jax import lax
import jax.experimental.pallas as pl
import jax.experimental.pallas.tpu as pltpu

CFG = dict(rows=24, lanes=4, kvg=2, ahead=80, mid=11, vs=16, cuts=(0, 1280, 1536, 1792), compute=True, ml=8, tl=(2, 2, 2))
B, H, SK, D, M, DC, DFF = 8, 32, 4096, 128, 512, 512, 1792
F32, BF16, U32 = jnp.float32, jnp.bfloat16, jnp.uint32
NSEM = 5


def _dot(a, b):
    return jnp.dot(a, b, preferred_element_type=F32)


def _dot_nt(a, b):
    return lax.dot_general(a, b, (((1,), (1,)), ((), ())), preferred_element_type=F32)


def _layernorm(x):
    d = x - jnp.mean(x, axis=-1, keepdims=True)
    return d * lax.rsqrt(jnp.mean(d * d, axis=-1, keepdims=True) + 1e-5)


def _head_tiles(w_ref, t, tmp_ref):
    rows = 128 * H
    tmp_ref[0:rows // 2, :] = pltpu.bitcast(w_ref[t * rows:(t + 1) * rows, :], U32)
    for j in range(H // 2):
        w = tmp_ref[pl.ds(j, 128, stride=H // 2), :]
        yield 2 * j, lax.bitcast_convert_type(w << 16, F32).astype(BF16)
        yield 2 * j + 1, lax.bitcast_convert_type(w & U32(0xFFFF0000), F32).astype(BF16)


class _Loader:
    def __init__(self, sems, order_sem):
        self.sems, self.order_sem = sems, order_sem
        self.pieces = []
        self.bufs = []
        self.end = []
        self.sem_of = {}
        self.free = list(range(NSEM))
        self.started = 0

    def add(self, *arrays):
        lanes, ids = [], []
        for src, dst, rows, n_lanes in arrays:
            ids.append(len(self.bufs))
            self.bufs.append(dst)
            span = src.shape[0] // n_lanes
            for lo in range(0, src.shape[0], span):
                cuts = [pl.ds(r, min(rows, lo + span - r)) for r in range(lo, lo + span, rows)]
                lanes.append([(ids[-1], src.at[s], dst.at[s]) for s in cuts])
        order = sorted(((k + 0.5) / len(lane), i, k) for i, lane in enumerate(lanes) for k in range(len(lane)))
        self.pieces += [lanes[i][k] for _, i, k in order]
        self.end += [len(self.pieces)] * len(arrays)
        return ids

    def start_until(self, n):
        while self.started < min(n, len(self.pieces)):
            buf, src, dst = self.pieces[self.started]
            if buf not in self.sem_of:
                self.sem_of[buf] = self.free.pop(0)
            pltpu.make_async_copy(src, dst, self.sems.at[self.sem_of[buf]]).start(priority=self.started % 2)
            self.started += 1

    def start_some(self, n):
        pl.semaphore_signal(self.order_sem, 1)
        pl.semaphore_wait(self.order_sem, 1)
        self.start_until(self.started + n)

    def wait(self, *ids):
        for buf in ids:
            self.start_until(self.end[buf] + CFG['ahead'])
        for buf in ids:
            sem = self.sem_of.pop(buf)
            pltpu.make_async_copy(self.bufs[buf], self.bufs[buf], self.sems.at[sem]).wait()
            self.free.append(sem)


def _kernel(x_hbm, c_hbm, kv_hbm, wq_hbm, wuk_hbm, wuv_hbm, wo_hbm, w1_hbm, w2_hbm, wm_hbm, o_ref,
            x_v, c_v, kv_v, wq_v, wuk_v, wuv_v, wo_v, w1_v, w2_v, wma_v, wmb_v,
            tmp_s, qa_s, cc_s, y_s, a_s, sems, order_sem):
    R, L, G = CFG['rows'], CFG['lanes'], CFG['kvg']
    cuts = list(zip(CFG['cuts'][:-1], CFG['cuts'][1:]))
    ld = _Loader(sems, order_sem)
    i_cx = ld.add((c_hbm, c_v, B, 1), (x_hbm, x_v, B, 1))
    i_wma = ld.add((wm_hbm.at[:, 0:3 * M], wma_v, 8, CFG['ml']))
    i_wqk = ld.add((wq_hbm, wq_v, 4 * R, L), (wuk_hbm, wuk_v, 4 * R, L))
    i_kv = [ld.add((kv_hbm.at[g * SK:(g + G) * SK], kv_v.at[g * SK:(g + G) * SK], R, G * L)) for g in range(0, B, G)]
    i_wvo = ld.add((wuv_hbm, wuv_v, 4 * R, L), (wo_hbm, wo_v, R, L))
    tl = CFG['tl']
    i_wmb, i_w1 = ld.add((wm_hbm.at[:, 3 * M:6 * M], wmb_v, 8, tl[0]), (w1_hbm, w1_v, 8, tl[1]))
    i_w2 = [ld.add((w2_hbm.at[lo:hi], w2_v.at[lo:hi], R, tl[2])) for lo, hi in cuts]
    step = -(-SK // L // R) * L // 4
    comp = CFG['compute']

    ld.wait(*i_cx)
    cf = c_v[...].astype(F32)
    sc = (cf * jax.nn.sigmoid(cf)).astype(BF16)
    x = x_v[...].astype(F32)
    ld.wait(*i_wma)
    mod_a = _dot(sc, wma_v[...])
    h = (_layernorm(x) * (1.0 + mod_a[:, M:2 * M]) + mod_a[:, 0:M]).astype(BF16)

    ld.wait(*i_wqk)
    if comp:
        q = [None] * H
        for t in range(4):
            for hd, w in _head_tiles(wq_v, t, tmp_s):
                part = _dot(h[:, t * 128:(t + 1) * 128], w)
                q[hd] = part if t == 0 else q[hd] + part
                if hd == CFG['mid']:
                    ld.start_some(step // 2)
            ld.start_some(step - step // 2)
        q = [(v * (D ** -0.5)).astype(BF16) for v in q]
        for t in range(4):
            for hd, w in _head_tiles(wuk_v, t, tmp_s):
                qa_s[t, pl.ds(hd, B, stride=H), :] = _dot_nt(q[hd], w)
                if hd == CFG['mid']:
                    ld.start_some(step // 2)
            ld.start_some(step - step // 2)

    for b in range(B):
        if b % G == 0:
            ld.wait(*i_kv[b // G])
        if not comp:
            continue
        if b + G >= B and b % G >= 2:
            step = 0
        heads = slice(b * H, (b + 1) * H)
        lo, hi = pl.ds(b * SK, SK // 2), pl.ds(b * SK + SK // 2, SK // 2)
        qa = jnp.concatenate([qa_s[t, heads, :] for t in range(4)], axis=1).astype(BF16)
        s0 = _dot_nt(qa, kv_v[lo, :])
        ld.start_some(step)
        s1 = _dot_nt(qa, kv_v[hi, :])
        ld.start_some(step)
        m = jnp.maximum(jnp.max(s0, axis=-1, keepdims=True), jnp.max(s1, axis=-1, keepdims=True))
        p0 = jnp.exp(s0 - m)
        cc = _dot(p0.astype(BF16), kv_v[lo, :])
        ld.start_some(step)
        p1 = jnp.exp(s1 - m)
        cc = cc + _dot(p1.astype(BF16), kv_v[hi, :])
        cc = cc * (1.0 / (jnp.sum(p0, axis=-1, keepdims=True) + jnp.sum(p1, axis=-1, keepdims=True)))
        for t in range(4):
            cc_s[t, heads, :] = cc[:, t * 128:(t + 1) * 128]
        ld.start_some(step)

    ld.wait(*i_wvo)
    att = x
    if comp:
        ctx = [None] * H
        for t in range(4):
            for hd, w in _head_tiles(wuv_v, t, tmp_s):
                part = _dot(cc_s[t, pl.ds(hd, B, stride=H), :].astype(BF16), w)
                ctx[hd] = part if t == 0 else ctx[hd] + part
                if hd == CFG['mid']:
                    ld.start_some(CFG['vs'])
            ld.start_some(CFG['vs'])
        att = _dot(jnp.concatenate(ctx, axis=1).astype(BF16), wo_v[...])
    y_s[0] = x + mod_a[:, 2 * M:3 * M] * att

    ld.start_some(len(ld.pieces))
    ld.wait(i_wmb, i_w1)
    mod_b = _dot(sc, wmb_v[...])
    y_s[1] = mod_b[:, 2 * M:3 * M]
    h2 = _layernorm(y_s[0]) * (1.0 + mod_b[:, M:2 * M]) + mod_b[:, 0:M]
    a_s[...] = jnp.maximum(_dot(h2.astype(BF16), w1_v[...]), 0.0)
    for i, (lo, hi) in enumerate(cuts):
        ld.wait(*i_w2[i])
        y = _dot(a_s[:, lo:hi].astype(BF16), w2_v[lo:hi, :])
        if i:
            y = y + y_s[2]
        if i + 1 < len(cuts):
            y_s[2] = y
    o_ref[...] = (y_s[0] + y_s[1] * y).astype(o_ref.dtype)
    assert not ld.sem_of and ld.started == len(ld.pieces)


@jax.jit
def pallas_adaLN_cond__compressed_kv_cla__dense_activation_relu__decode_kernel(
        A_x, A_c_kv, A_w_q, A_w_uk, A_w_uv, A_w_o, B_x, B_w1, B_w2, c, w_mod):
    del B_x
    hbm = pl.BlockSpec(memory_space=pl.ANY)
    out = pl.pallas_call(
        _kernel,
        in_specs=[hbm] * 10,
        out_specs=pl.BlockSpec(memory_space=pltpu.VMEM),
        out_shape=jax.ShapeDtypeStruct((B, M), A_x.dtype),
        scratch_shapes=[
            pltpu.VMEM((B, M), BF16), pltpu.VMEM((B, M), BF16), pltpu.VMEM((B * SK, DC), BF16),
            pltpu.VMEM((M * H, D), BF16), pltpu.VMEM((DC * H, D), BF16), pltpu.VMEM((DC * H, D), BF16),
            pltpu.VMEM((H * D, M), BF16), pltpu.VMEM((M, DFF), BF16), pltpu.VMEM((DFF, M), BF16),
            pltpu.VMEM((M, 3 * M), BF16), pltpu.VMEM((M, 3 * M), BF16),
            pltpu.VMEM((129 * H // 2, D), U32),
            pltpu.VMEM((4, (B + 1) * H, 128), F32), pltpu.VMEM((4, (B + 1) * H, 128), F32),
            pltpu.VMEM((3, B, M), F32), pltpu.VMEM((B, DFF), F32),
            pltpu.SemaphoreType.DMA((NSEM,)), pltpu.SemaphoreType.REGULAR,
        ],
        compiler_params=pltpu.CompilerParams(vmem_limit_bytes=100 * 1024 * 1024),
    )(A_x.reshape(B, M), c, A_c_kv.reshape(B * SK, DC), A_w_q.reshape(M * H, D), A_w_uk.reshape(DC * H, D),
      A_w_uv.reshape(DC * H, D), A_w_o.reshape(H * D, M), B_w1, B_w2, w_mod)
    return out.reshape(B, 1, M)
```

```python
import numpy as np
import jax
import jax.numpy as jnp
from jax import lax
import jax.experimental.pallas as pl
import jax.experimental.pallas.tpu as pltpu

B, H, SK, D, M, DC, DFF = 8, 32, 4096, 128, 512, 512, 1792
F32, BF16, U32 = jnp.float32, jnp.bfloat16, jnp.uint32

ROWS = 24
LANES = 4
KV_GROUP = 2
AHEAD = 80
BURST = 43
TAIL_BURST = 18
W2_CUTS = ((0, 1280), (1280, 1536), (1536, DFF))
NUM_SEMS = 5


def _dot(a, b):
    return jnp.dot(a, b, preferred_element_type=F32)


def _dot_nt(a, b):
    return lax.dot_general(a, b, (((1,), (1,)), ((), ())), preferred_element_type=F32)


def _layernorm(x):
    d = x - jnp.mean(x, axis=-1, keepdims=True)
    return d * lax.rsqrt(jnp.mean(d * d, axis=-1, keepdims=True) + 1e-5)


class _Loader:
    def __init__(self, sems, order_sem):
        self.sems, self.order_sem = sems, order_sem
        self.pieces = []
        self.dst = []
        self.end = []
        self.sem_of = {}
        self.free = list(range(NUM_SEMS))
        self.started = 0

    def add(self, *operands):
        lanes, ids = [], []
        for src, dst, rows, n_lanes in operands:
            ids.append(len(self.dst))
            self.dst.append(dst)
            span = src.shape[0] // n_lanes
            for lo in range(0, src.shape[0], span):
                cuts = [pl.ds(r, min(rows, lo + span - r)) for r in range(lo, lo + span, rows)]
                lanes.append([(ids[-1], src.at[s], dst.at[s]) for s in cuts])
        order = sorted(((k + 0.5) / len(lane), i, k)
                       for i, lane in enumerate(lanes) for k in range(len(lane)))
        self.pieces += [lanes[i][k] for _, i, k in order]
        self.end += [len(self.pieces)] * len(operands)
        return ids

    def _start_until(self, n):
        while self.started < min(n, len(self.pieces)):
            op, src, dst = self.pieces[self.started]
            if op not in self.sem_of:
                self.sem_of[op] = self.free.pop(0)
            copy = pltpu.make_async_copy(src, dst, self.sems.at[self.sem_of[op]])
            copy.start(priority=self.started % 2)
            self.started += 1

    def burst(self, n):
        pl.semaphore_signal(self.order_sem, 1)
        pl.semaphore_wait(self.order_sem, 1)
        self._start_until(self.started + n)

    def wait(self, ids):
        self._start_until(max(self.end[op] for op in ids) + AHEAD)
        for op in ids:
            sem = self.sem_of.pop(op)
            pltpu.make_async_copy(self.dst[op], self.dst[op], self.sems.at[sem]).wait()
            self.free.append(sem)


def _head_tiles(w_ref, pair_ref, loader, burst):
    rows = 128 * H
    for t in range(4):
        pair_ref[0:rows // 2, :] = pltpu.bitcast(w_ref[t * rows:(t + 1) * rows, :], U32)
        for j in range(H // 2):
            w = pair_ref[pl.ds(j, 128, stride=H // 2), :]
            yield t, 2 * j, lax.bitcast_convert_type(w << 16, F32).astype(BF16)
            yield t, 2 * j + 1, lax.bitcast_convert_type(w & np.uint32(0xFFFF0000), F32).astype(BF16)
            if j == 5:
                loader.burst(burst // 2)
        loader.burst(burst - burst // 2)


def _kernel(x_hbm, c_hbm, kv_hbm, wq_hbm, wuk_hbm, wuv_hbm, wo_hbm, w1_hbm, w2_hbm, wm_hbm, o_ref,
            x_v, c_v, kv_v, wq_v, wuk_v, wuv_v, wo_v, w1_v, w2_v, wma_v, wmb_v,
            pair_s, qa_s, cc_s, x1_s, gb_s, act_s, y_s):

    def stream(sems, order_sem):
        ld = _Loader(sems, order_sem)
        i_cx = ld.add((c_hbm, c_v, B, 1), (x_hbm, x_v, B, 1))
        i_wma = ld.add((wm_hbm.at[:, 0:3 * M], wma_v, 8, 8))
        i_wqk = ld.add((wq_hbm, wq_v, 4 * ROWS, LANES), (wuk_hbm, wuk_v, 4 * ROWS, LANES))
        i_kv = []
        for b in range(0, B, KV_GROUP):
            keys = pl.ds(b * SK, KV_GROUP * SK)
            i_kv.append(ld.add((kv_hbm.at[keys], kv_v.at[keys], ROWS, KV_GROUP * LANES)))
        i_wvo = ld.add((wuv_hbm, wuv_v, 4 * ROWS, LANES), (wo_hbm, wo_v, ROWS, LANES))
        i_ffn = ld.add((wm_hbm.at[:, 3 * M:6 * M], wmb_v, 8, 2), (w1_hbm, w1_v, 8, 2))
        i_w2 = [ld.add((w2_hbm.at[lo:hi], w2_v.at[lo:hi], ROWS, 2)) for lo, hi in W2_CUTS]

        ld.wait(i_cx)
        c = c_v[...].astype(F32)
        silu_c = (c * jax.nn.sigmoid(c)).astype(BF16)
        x = x_v[...].astype(F32)
        pair_s[64 * H:, :] = jnp.zeros((H // 2, D), U32)
        qa_s[:, B * H:, :] = jnp.zeros((4, H, 128), F32)
        cc_s[:, B * H:, :] = jnp.zeros((4, H, 128), F32)
        ld.wait(i_wma)
        mod_a = _dot(silu_c, wma_v[...])
        h = (_layernorm(x) * (1.0 + mod_a[:, M:2 * M]) + mod_a[:, 0:M]).astype(BF16)

        ld.wait(i_wqk)
        q = [None] * H
        for t, head, w in _head_tiles(wq_v, pair_s, ld, BURST):
            part = _dot(h[:, t * 128:(t + 1) * 128], w)
            q[head] = part if t == 0 else q[head] + part
        q = [(v * D ** -0.5).astype(BF16) for v in q]
        for t, head, w in _head_tiles(wuk_v, pair_s, ld, BURST):
            qa_s[t, pl.ds(head, B, stride=H), :] = _dot_nt(q[head], w)

        for b in range(B):
            if b % KV_GROUP == 0:
                ld.wait(i_kv[b // KV_GROUP])
            heads = pl.ds(b * H, H)
            lo, hi = pl.ds(b * SK, SK // 2), pl.ds(b * SK + SK // 2, SK // 2)
            qa = jnp.concatenate([qa_s[t, heads, :] for t in range(4)], axis=1).astype(BF16)
            s0 = _dot_nt(qa, kv_v[lo, :])
            ld.burst(BURST)
            s1 = _dot_nt(qa, kv_v[hi, :])
            ld.burst(BURST)
            m = jnp.maximum(jnp.max(s0, axis=-1, keepdims=True), jnp.max(s1, axis=-1, keepdims=True))
            p0 = jnp.exp(s0 - m)
            cc = _dot(p0.astype(BF16), kv_v[lo, :])
            ld.burst(BURST)
            p1 = jnp.exp(s1 - m)
            cc = cc + _dot(p1.astype(BF16), kv_v[hi, :])
            denom = jnp.sum(p0, axis=-1, keepdims=True) + jnp.sum(p1, axis=-1, keepdims=True)
            cc = cc * (1.0 / denom)
            for t in range(4):
                cc_s[t, heads, :] = cc[:, t * 128:(t + 1) * 128]
            ld.burst(BURST)

        ld.wait(i_wvo)
        ctx = [None] * H
        for t, head, w in _head_tiles(wuv_v, pair_s, ld, 2 * TAIL_BURST):
            part = _dot(cc_s[t, pl.ds(head, B, stride=H), :].astype(BF16), w)
            ctx[head] = part if t == 0 else ctx[head] + part
        att = _dot(jnp.concatenate(ctx, axis=1).astype(BF16), wo_v[...])
        x1_s[...] = x + mod_a[:, 2 * M:3 * M] * att
        ld.burst(len(ld.pieces))

        ld.wait(i_ffn)
        mod_b = _dot(silu_c, wmb_v[...])
        gb_s[...] = mod_b[:, 2 * M:3 * M]
        h2 = _layernorm(x1_s[...]) * (1.0 + mod_b[:, M:2 * M]) + mod_b[:, 0:M]
        act_s[...] = jnp.maximum(_dot(h2.astype(BF16), w1_v[...]), 0.0)
        for i, (lo, hi) in enumerate(W2_CUTS[:-1]):
            ld.wait(i_w2[i])
            y = _dot(act_s[:, lo:hi].astype(BF16), w2_v[lo:hi, :])
            y_s[...] = y if i == 0 else y_s[...] + y
        ld.wait(i_w2[-1])
        assert not ld.sem_of and ld.started == len(ld.pieces)

    pl.run_scoped(stream, pltpu.SemaphoreType.DMA((NUM_SEMS,)), pltpu.SemaphoreType.REGULAR)
    lo, hi = W2_CUTS[-1]
    y = y_s[...] + _dot(act_s[:, lo:hi].astype(BF16), w2_v[lo:hi, :])
    o_ref[...] = (x1_s[...] + gb_s[...] * y).astype(o_ref.dtype)


@jax.jit
def pallas_adaLN_cond__compressed_kv_cla__dense_activation_relu__decode_kernel(
    A_x: jax.Array,
    A_c_kv: jax.Array,
    A_w_q: jax.Array,
    A_w_uk: jax.Array,
    A_w_uv: jax.Array,
    A_w_o: jax.Array,
    B_x: jax.Array,
    B_w1: jax.Array,
    B_w2: jax.Array,
    c: jax.Array,
    w_mod: jax.Array,
):
    del B_x
    out = pl.pallas_call(
        _kernel,
        in_specs=[pl.BlockSpec(memory_space=pl.ANY)] * 10,
        out_specs=pl.BlockSpec(memory_space=pltpu.VMEM),
        out_shape=jax.ShapeDtypeStruct((B, M), A_x.dtype),
        scratch_shapes=[
            pltpu.VMEM((B, M), BF16),
            pltpu.VMEM((B, M), BF16),
            pltpu.VMEM((B * SK, DC), BF16),
            pltpu.VMEM((M * H, D), BF16),
            pltpu.VMEM((DC * H, D), BF16),
            pltpu.VMEM((DC * H, D), BF16),
            pltpu.VMEM((H * D, M), BF16),
            pltpu.VMEM((M, DFF), BF16),
            pltpu.VMEM((DFF, M), BF16),
            pltpu.VMEM((M, 3 * M), BF16),
            pltpu.VMEM((M, 3 * M), BF16),
            pltpu.VMEM((129 * H // 2, D), U32),
            pltpu.VMEM((4, (B + 1) * H, 128), F32),
            pltpu.VMEM((4, (B + 1) * H, 128), F32),
            pltpu.VMEM((B, M), F32),
            pltpu.VMEM((B, M), F32),
            pltpu.VMEM((B, DFF), F32),
            pltpu.VMEM((B, M), F32),
        ],
        compiler_params=pltpu.CompilerParams(vmem_limit_bytes=100 * 1024 * 1024),
    )(A_x.reshape(B, M), c, A_c_kv.reshape(B * SK, DC), A_w_q.reshape(M * H, D),
      A_w_uk.reshape(DC * H, D), A_w_uv.reshape(DC * H, D), A_w_o.reshape(H * D, M),
      B_w1, B_w2, w_mod)
    return out.reshape(B, 1, M)
```
